```python
import os as _os
_os.environ.setdefault("JAX_PLATFORMS", "cpu")
import jax
import jax.numpy as jnp

def _softmax(x, axis=-1):
    return jax.nn.softmax(x, axis=axis)
def _gelu(x):
    return jax.nn.gelu(x, approximate=True)
def _silu(x):
    return jax.nn.silu(x)
def _sigmoid(x):
    return jax.nn.sigmoid(x)
def _layernorm(x, axis=-1, eps=1e-5):
    m = jnp.mean(x, axis=axis, keepdims=True)
    v = jnp.var(x, axis=axis, keepdims=True)
    return (x - m) / jnp.sqrt(v + eps)
def _scatter_add(tgt, idx, src, axis=0):
    return tgt.at[idx].add(src)
def _segment_sum(src, seg, n):
    return jax.ops.segment_sum(src, seg, n)
class _Rng:
    def __init__(self, key):
        self._k = key
    def _next(self):
        self._k, sub = jax.random.split(self._k)
        return sub
    def normal(self, shape):
        return jax.random.normal(self._next(), shape, dtype=jnp.bfloat16)
    def randint(self, lo, hi, shape):
        return jax.random.randint(self._next(), shape, lo, hi, dtype=jnp.int32)
    def uniform(self, shape, lo=0.0, hi=1.0):
        return jax.random.uniform(self._next(), shape, jnp.bfloat16, lo, hi)
    def permutation(self, n):
        return jax.random.permutation(self._next(), n)


kernel_name = 'concat_heads__mha_block_cached__mha_block_cached__near_ridge'

def setup_inputs():
    _rng = _Rng(jax.random.key(int.from_bytes(__import__("os").urandom(4), "little")))
    _w = (lambda a: (lambda t: t.astype(jnp.bfloat16) if jnp.issubdtype(t.dtype, jnp.floating) else t)(jnp.asarray(a)))
    def _A_setup():
        B, Sq, D = 8, 160, 512
        H, Sk, Dh = 32, 512, 128
        return {
            "x": _w((lambda *s: _rng.normal(s) * 0.8)(B, Sq, D)),
            "k_cache": _w((lambda *s: _rng.normal(s) * 0.8)(B, H, Sk, Dh)),
            "v_cache": _w((lambda *s: _rng.normal(s) * 0.05)(B, H, Sk, Dh)),
            "wq": _w((lambda *s: _rng.normal(s) * 0.8)(D, H * Dh) * (D ** -0.5)),
            "wo": _w((lambda *s: _rng.normal(s) * 0.05)(H * Dh, D) * ((H * Dh) ** -0.5)),
        }
    _A_in = _A_setup()

    def _B_setup():
        B, Sq, D = 8, 160, 512
        H, Sk, Dh = 32, 512, 128
        return {
            "x": _w((lambda *s: _rng.normal(s) * 0.8)(B, Sq, D)),
            "k_cache": _w((lambda *s: _rng.normal(s) * 0.8)(B, H, Sk, Dh)),
            "v_cache": _w((lambda *s: _rng.normal(s) * 0.05)(B, H, Sk, Dh)),
            "wq": _w((lambda *s: _rng.normal(s) * 0.8)(D, H * Dh) * (D ** -0.5)),
            "wo": _w((lambda *s: _rng.normal(s) * 0.05)(H * Dh, D) * ((H * Dh) ** -0.5)),
        }
    _B_in = _B_setup()

    return {
        "A_x": _A_in["x"],
        "A_k_cache": _A_in["k_cache"],
        "A_v_cache": _A_in["v_cache"],
        "A_wq": _A_in["wq"],
        "A_wo": _A_in["wo"],
        "B_x": _B_in["x"],
        "B_k_cache": _B_in["k_cache"],
        "B_v_cache": _B_in["v_cache"],
        "B_wq": _B_in["wq"],
        "B_wo": _B_in["wo"],
    }

def reference(A_x, A_k_cache, A_v_cache, A_wq, A_wo, B_x, B_k_cache, B_v_cache, B_wq, B_wo):
    def _A_ref(x, k_cache, v_cache, wq, wo):
        B, Sq, D = x.shape
        H, Dh = 32, 128
        q = (lambda x, *d: x.transpose(*d))((x @ wq).reshape(B, Sq, H, Dh), 0, 2, 1, 3)
        scores = jnp.einsum("bhqd,bhkd->bhqk", q, k_cache) * (Dh ** -0.5)
        p = _softmax(scores, axis=-1)
        o = jnp.einsum("bhqk,bhkd->bhqd", p, v_cache)
        return (lambda x, *d: x.transpose(*d))(o, 0, 2, 1, 3).reshape(B, Sq, H * Dh) @ wo

    def _B_ref(x, k_cache, v_cache, wq, wo):
        B, Sq, D = x.shape
        H, Dh = 32, 128
        q = (lambda x, *d: x.transpose(*d))((x @ wq).reshape(B, Sq, H, Dh), 0, 2, 1, 3)
        scores = jnp.einsum("bhqd,bhkd->bhqk", q, k_cache) * (Dh ** -0.5)
        p = _softmax(scores, axis=-1)
        o = jnp.einsum("bhqk,bhkd->bhqd", p, v_cache)
        return (lambda x, *d: x.transpose(*d))(o, 0, 2, 1, 3).reshape(B, Sq, H * Dh) @ wo

    a = _A_ref(A_x, A_k_cache, A_v_cache, A_wq, A_wo)
    b = _B_ref(B_x, B_k_cache, B_v_cache, B_wq, B_wo)
    return jnp.concatenate([a, b], axis=-1)
```

```python
import functools
import jax
import jax.numpy as jnp
from jax import lax
import jax.experimental.pallas as pl
import jax.experimental.pallas.tpu as pltpu

HB = 8


@jax.jit
def pallas_concat_heads__mha_block_cached__mha_block_cached__near_ridge_kernel(
    A_x: jax.Array,
    A_k_cache: jax.Array,
    A_v_cache: jax.Array,
    A_wq: jax.Array,
    A_wo: jax.Array,
    B_x: jax.Array,
    B_k_cache: jax.Array,
    B_v_cache: jax.Array,
    B_wq: jax.Array,
    B_wo: jax.Array,
):
    B, Sq, D = A_x.shape
    _, H, Sk, Dh = A_k_cache.shape
    hb = HB
    nh = H // hb
    scale = float(Dh) ** -0.5
    f32 = jnp.float32
    bf16 = jnp.bfloat16

    def kernel(xa_ref, ka_ref, va_ref, wqa_ref, woa_ref,
               xb_ref, kb_ref, vb_ref, wqb_ref, wob_ref,
               o_ref, acc_ref):
        ab = pl.program_id(0)
        hblk = pl.program_id(1)
        b = pl.program_id(2)

        def body(x_ref, k_ref, v_ref, wq_ref, wo_ref):
            x = x_ref[b]
            q = jnp.dot(x, wq_ref[...], preferred_element_type=f32).astype(bf16)
            outs = []
            for h in range(hb):
                qh = q[:, h * Dh:(h + 1) * Dh]
                s = lax.dot_general(qh, k_ref[0, h], (((1,), (1,)), ((), ())),
                                    preferred_element_type=f32)
                m = jnp.max(s, axis=-1, keepdims=True)
                p = jnp.exp((s - m) * scale)
                l = jnp.sum(p, axis=-1, keepdims=True)
                o = jnp.dot(p.astype(bf16), v_ref[0, h], preferred_element_type=f32)
                outs.append((o * (1.0 / l)).astype(bf16))
            o_all = jnp.concatenate(outs, axis=-1)
            contrib = jnp.dot(o_all, wo_ref[...], preferred_element_type=f32)

            @pl.when(hblk == 0)
            def _():
                acc_ref[b] = contrib

            @pl.when(hblk > 0)
            def _():
                acc_ref[b] += contrib

            @pl.when(hblk == nh - 1)
            def _():
                o_ref[b] = acc_ref[b].astype(o_ref.dtype)

        @pl.when(ab == 0)
        def _():
            body(xa_ref, ka_ref, va_ref, wqa_ref, woa_ref)

        @pl.when(ab == 1)
        def _():
            body(xb_ref, kb_ref, vb_ref, wqb_ref, wob_ref)

    def kv_map(which):
        if which == 0:
            return lambda ab, h, b: (jnp.where(ab == 0, b, B - 1), jnp.where(ab == 0, h, nh - 1), 0, 0)
        return lambda ab, h, b: (jnp.where(ab == 1, b, 0), jnp.where(ab == 1, h, 0), 0, 0)

    def wq_map(which):
        if which == 0:
            return lambda ab, h, b: (0, jnp.where(ab == 0, h, nh - 1))
        return lambda ab, h, b: (0, jnp.where(ab == 1, h, 0))

    def wo_map(which):
        if which == 0:
            return lambda ab, h, b: (jnp.where(ab == 0, h, nh - 1), 0)
        return lambda ab, h, b: (jnp.where(ab == 1, h, 0), 0)

    def specs(which):
        return [
            pl.BlockSpec((B, Sq, D), lambda ab, h, b: (0, 0, 0)),
            pl.BlockSpec((1, hb, Sk, Dh), kv_map(which)),
            pl.BlockSpec((1, hb, Sk, Dh), kv_map(which)),
            pl.BlockSpec((D, hb * Dh), wq_map(which)),
            pl.BlockSpec((hb * Dh, D), wo_map(which)),
        ]

    return pl.pallas_call(
        kernel,
        grid=(2, nh, B),
        in_specs=specs(0) + specs(1),
        out_specs=pl.BlockSpec((B, Sq, D), lambda ab, h, b: (0, 0, ab)),
        out_shape=jax.ShapeDtypeStruct((B, Sq, 2 * D), A_x.dtype),
        scratch_shapes=[pltpu.VMEM((B, Sq, D), f32)],
        compiler_params=pltpu.CompilerParams(
            dimension_semantics=("arbitrary", "arbitrary", "arbitrary"),
            vmem_limit_bytes=100 * 1024 * 1024,
        ),
    )(A_x, A_k_cache, A_v_cache, A_wq, A_wo, B_x, B_k_cache, B_v_cache, B_wq, B_wo)
```

```python
import functools
import jax
import jax.numpy as jnp
from jax import lax
import jax.experimental.pallas as pl
import jax.experimental.pallas.tpu as pltpu
HB = 8
NB = 4
LA_ENV = 1
NW = 4
LOG2E = 1.4426950408889634


@jax.jit
def pallas_concat_heads__mha_block_cached__mha_block_cached__near_ridge_kernel(
    A_x, A_k_cache, A_v_cache, A_wq, A_wo, B_x, B_k_cache, B_v_cache, B_wq, B_wo,
):
    B, Sq, D = A_x.shape
    _, H, Sk, Dh = A_k_cache.shape
    hb = HB
    assert hb >= 3
    nh = H // hb
    nsteps = nh * B
    scale = float(Dh) ** -0.5
    f32 = jnp.float32
    bf16 = jnp.bfloat16
    wq_rows = D // B
    wo_rows = (hb * Dh) // B
    LA = LA_ENV
    assert B & (B - 1) == 0
    LB = B.bit_length() - 1

    def kernel(xa_hbm, ka_hbm, va_hbm, wqa_hbm, woa_hbm,
               xb_hbm, kb_hbm, vb_hbm, wqb_hbm, wob_hbm,
               o_hbm,
               x_s, wq_s, wo_s, k_s, v_s, acc_s, o_s, q_c, s_c, o_c,
               sem_x, sem_w, sem_kv, sem_o):
        x_hbm = (xa_hbm, xb_hbm)
        k_hbm = (ka_hbm, kb_hbm)
        v_hbm = (va_hbm, vb_hbm)
        wq_hbm = (wqa_hbm, wqb_hbm)
        wo_hbm = (woa_hbm, wob_hbm)

        def kv_copies(step, slot):
            hblk = step >> LB
            b = step & (B - 1)
            cps = []
            for w in range(2):
                cps.append(pltpu.make_async_copy(
                    k_hbm[w].at[b, pl.ds(hblk * hb, hb)], k_s.at[slot, w], sem_kv.at[slot, 2 * w]))
                cps.append(pltpu.make_async_copy(
                    v_hbm[w].at[b, pl.ds(hblk * hb, hb)], v_s.at[slot, w], sem_kv.at[slot, 2 * w + 1]))
            return cps

        def x_copy(w, b):
            return pltpu.make_async_copy(x_hbm[w].at[b], x_s.at[w, b], sem_x.at[w, b])

        def w_piece_copies(hblk, wslot, piece):
            cps = []
            for w in range(2):
                cps.append(pltpu.make_async_copy(
                    wq_hbm[w].at[pl.ds(piece * wq_rows, wq_rows), pl.ds(hblk * hb * Dh, hb * Dh)],
                    wq_s.at[wslot, w, pl.ds(piece * wq_rows, wq_rows)],
                    sem_w.at[wslot, 2 * w]))
                cps.append(pltpu.make_async_copy(
                    wo_hbm[w].at[pl.ds(hblk * hb * Dh + piece * wo_rows, wo_rows)],
                    wo_s.at[wslot, w, pl.ds(piece * wo_rows, wo_rows)],
                    sem_w.at[wslot, 2 * w + 1]))
            return cps

        def w_wait(wslot):
            for w in range(2):
                pltpu.make_async_copy(wq_s.at[wslot, w], wq_s.at[wslot, w], sem_w.at[wslot, 2 * w]).wait()
                pltpu.make_async_copy(wo_s.at[wslot, w], wo_s.at[wslot, w], sem_w.at[wslot, 2 * w + 1]).wait()

        def o_copy(b):
            return pltpu.make_async_copy(o_s.at[b], o_hbm.at[b], sem_o.at[b])

        def finalize(b):
            o_s[b, :, 0:D] = acc_s[0, b].astype(o_s.dtype)
            o_s[b, :, D:2 * D] = acc_s[1, b].astype(o_s.dtype)
            o_copy(b).start()

        x_copy(0, 0).start()
        x_copy(1, 0).start()
        for piece in range(B):
            for c in w_piece_copies(0, 0, piece):
                c.start()
        for c in kv_copies(0, 0):
            c.start()
        q_c[...] = jnp.zeros(q_c.shape, q_c.dtype)
        s_c[...] = jnp.zeros(s_c.shape, s_c.dtype)
        o_c[...] = jnp.zeros(o_c.shape, o_c.dtype)
        acc_s[1, B] = jnp.zeros((Sq, D), f32)

        tasks = [(w, h) for w in range(2) for h in range(hb)]
        T = len(tasks)

        def make_stages(ctx, q, s, p, l, o):
            def S1(t):
                w, h, slot, wslot, b = ctx(t)
                q[t] = jnp.dot(x_s[w, b], wq_s[wslot, w, :, h * Dh:(h + 1) * Dh],
                               preferred_element_type=f32).astype(bf16)

            def S2(t):
                w, h, slot, wslot, b = ctx(t)
                s[t] = lax.dot_general(q.pop(t), k_s[slot, w, h], (((1,), (1,)), ((), ())),
                                       preferred_element_type=f32)

            def S3(t):
                st = s.pop(t)
                m = jnp.max(st, axis=-1, keepdims=True)
                pt = jnp.exp2((st - m) * (scale * LOG2E))
                l[t] = jnp.sum(pt, axis=-1, keepdims=True)
                p[t] = pt.astype(bf16)

            def S4(t):
                w, h, slot, wslot, b = ctx(t)
                ot = jnp.dot(p.pop(t), v_s[slot, w, h], preferred_element_type=f32)
                o[t] = (ot * (1.0 / l.pop(t))).astype(bf16)

            def S5(t):
                w, h, slot, wslot, b = ctx(t)
                acc_s[w, b] += jnp.dot(o.pop(t), wo_s[wslot, w, h * Dh:(h + 1) * Dh, :],
                                       preferred_element_type=f32)
            return S1, S2, S3, S4, S5

        def step_body(step, carry):
            hblk = step >> LB
            b = step & (B - 1)
            slot = step & (NB - 1)
            wslot = hblk & (NW - 1)
            pstep = jnp.maximum(step - 1, 0)
            phblk = pstep >> LB
            pslot = pstep & (NB - 1)
            pwslot = phblk & (NW - 1)
            pb = jnp.where(step == 0, B, pstep & (B - 1))

            @pl.when(b == 0)
            def _():
                w_wait(wslot)

            @pl.when(hblk == 0)
            def _():
                x_copy(0, b).wait()
                x_copy(1, b).wait()
                acc_s[0, b] = jnp.zeros((Sq, D), f32)
                acc_s[1, b] = jnp.zeros((Sq, D), f32)

            for c in kv_copies(step, slot):
                c.wait()

            if LA == 1:
                @pl.when(step + 1 < nsteps)
                def _():
                    for c in kv_copies(step + 1, (step + 1) & (NB - 1)):
                        c.start()
            else:
                @pl.when(step == 0)
                def _():
                    for la in range(1, LA):
                        for c in kv_copies(la, la % NB):
                            c.start()

                @pl.when(step + LA < nsteps)
                def _():
                    for c in kv_copies(step + LA, (step + LA) & (NB - 1)):
                        c.start()

            @pl.when(jnp.logical_and(hblk == 0, b + 1 < B))
            def _():
                x_copy(0, b + 1).start()
                x_copy(1, b + 1).start()

            @pl.when(hblk + 1 < nh)
            def _():
                for c in w_piece_copies(hblk + 1, (hblk + 1) & (NW - 1), b):
                    c.start()

            def ctx(t):
                if t < 0:
                    return (1, hb + t, pslot, pwslot, pb)
                w, h = tasks[t]
                return (w, h, slot, wslot, b)

            q = {-1: q_c[...]}; s = {-2: s_c[...]}; p = {}; l = {}; o = {-3: o_c[...]}
            S1, S2, S3, S4, S5 = make_stages(ctx, q, s, p, l, o)
            for i in range(T):
                S1(i); S2(i - 1); S3(i - 2); S4(i - 2); S5(i - 3)
            q_c[...] = q.pop(T - 1)
            s_c[...] = s.pop(T - 2)
            o_c[...] = o.pop(T - 3)

            @pl.when(jnp.logical_and(step > 0, phblk == nh - 1))
            def _():
                finalize(pb)

            return carry

        lax.fori_loop(0, nsteps, step_body, 0)

        last = nsteps - 1

        def ctx_l(t):
            return (1, hb + t, last % NB, (nh - 1) % NW, B - 1)

        q = {-1: q_c[...]}; s = {-2: s_c[...]}; p = {}; l = {}; o = {-3: o_c[...]}
        S1, S2, S3, S4, S5 = make_stages(ctx_l, q, s, p, l, o)
        S2(-1); S3(-2); S4(-2); S5(-3)
        S3(-1); S4(-1); S5(-2)
        S5(-1)
        finalize(B - 1)

        for b in range(B):
            o_copy(b).wait()

    any_spec = pl.BlockSpec(memory_space=pl.ANY)
    return pl.pallas_call(
        kernel,
        in_specs=[any_spec] * 10,
        out_specs=any_spec,
        out_shape=jax.ShapeDtypeStruct((B, Sq, 2 * D), A_x.dtype),
        scratch_shapes=[
            pltpu.VMEM((2, B, Sq, D), bf16),
            pltpu.VMEM((NW, 2, D, hb * Dh), bf16),
            pltpu.VMEM((NW, 2, hb * Dh, D), bf16),
            pltpu.VMEM((NB, 2, hb, Sk, Dh), bf16),
            pltpu.VMEM((NB, 2, hb, Sk, Dh), bf16),
            pltpu.VMEM((2, B + 1, Sq, D), f32),
            pltpu.VMEM((B, Sq, 2 * D), bf16),
            pltpu.VMEM((Sq, Dh), bf16),
            pltpu.VMEM((Sq, Sk), f32),
            pltpu.VMEM((Sq, Dh), bf16),
            pltpu.SemaphoreType.DMA((2, B)),
            pltpu.SemaphoreType.DMA((NW, 4)),
            pltpu.SemaphoreType.DMA((NB, 4)),
            pltpu.SemaphoreType.DMA((B,)),
        ],
        compiler_params=pltpu.CompilerParams(
            vmem_limit_bytes=100 * 1024 * 1024, disable_bounds_checks=True,
        ),
    )(A_x, A_k_cache, A_v_cache, A_wq, A_wo, B_x, B_k_cache, B_v_cache, B_wq, B_wo)
```

```python
import jax
import jax.numpy as jnp
from jax import lax
import jax.experimental.pallas as pl
import jax.experimental.pallas.tpu as pltpu

HB = 4
BB = 2
NB = 4
NW = 4
LOG2E = 1.4426950408889634


@jax.jit
def pallas_concat_heads__mha_block_cached__mha_block_cached__near_ridge_kernel(
    A_x, A_k_cache, A_v_cache, A_wq, A_wo, B_x, B_k_cache, B_v_cache, B_wq, B_wo,
):
    B, Sq, D = A_x.shape
    _, H, Sk, Dh = A_k_cache.shape
    hb, bb = HB, BB
    assert hb >= 4
    nh = H // hb
    nbp = B // bb
    nsteps = nh * nbp
    scale = float(Dh) ** -0.5
    f32 = jnp.float32
    bf16 = jnp.bfloat16
    wq_rows = D // nbp
    wo_rows = (hb * Dh) // nbp
    assert nbp & (nbp - 1) == 0
    LB = nbp.bit_length() - 1

    def kernel(xa_hbm, ka_hbm, va_hbm, wqa_hbm, woa_hbm,
               xb_hbm, kb_hbm, vb_hbm, wqb_hbm, wob_hbm,
               o_hbm,
               x_s, wq_s, wo_s, k_s, v_s, acc_s, o_s, q_c, s_c, o_c,
               sem_x, sem_w, sem_kv, sem_o):
        x_hbm = (xa_hbm, xb_hbm)
        k_hbm = (ka_hbm, kb_hbm)
        v_hbm = (va_hbm, vb_hbm)
        wq_hbm = (wqa_hbm, wqb_hbm)
        wo_hbm = (woa_hbm, wob_hbm)

        def kv_copies(step, slot):
            hblk = step >> LB
            bp = step & (nbp - 1)
            cps = []
            for w in range(2):
                cps.append(pltpu.make_async_copy(
                    k_hbm[w].at[pl.ds(bp * bb, bb), pl.ds(hblk * hb, hb)], k_s.at[slot, w], sem_kv.at[slot, 2 * w]))
                cps.append(pltpu.make_async_copy(
                    v_hbm[w].at[pl.ds(bp * bb, bb), pl.ds(hblk * hb, hb)], v_s.at[slot, w], sem_kv.at[slot, 2 * w + 1]))
            return cps

        def x_copy(w, bp):
            return pltpu.make_async_copy(x_hbm[w].at[pl.ds(bp * bb, bb)], x_s.at[w, pl.ds(bp * bb, bb)], sem_x.at[w, bp])

        def w_piece_copies(hblk, wslot, piece):
            cps = []
            for w in range(2):
                cps.append(pltpu.make_async_copy(
                    wq_hbm[w].at[pl.ds(piece * wq_rows, wq_rows), pl.ds(hblk * hb * Dh, hb * Dh)],
                    wq_s.at[wslot, w, pl.ds(piece * wq_rows, wq_rows)],
                    sem_w.at[wslot, 2 * w]))
                cps.append(pltpu.make_async_copy(
                    wo_hbm[w].at[pl.ds(hblk * hb * Dh + piece * wo_rows, wo_rows)],
                    wo_s.at[wslot, w, pl.ds(piece * wo_rows, wo_rows)],
                    sem_w.at[wslot, 2 * w + 1]))
            return cps

        def w_wait(wslot):
            for w in range(2):
                pltpu.make_async_copy(wq_s.at[wslot, w], wq_s.at[wslot, w], sem_w.at[wslot, 2 * w]).wait()
                pltpu.make_async_copy(wo_s.at[wslot, w], wo_s.at[wslot, w], sem_w.at[wslot, 2 * w + 1]).wait()

        def o_copy(bp):
            return pltpu.make_async_copy(o_s.at[pl.ds(bp * bb, bb)], o_hbm.at[pl.ds(bp * bb, bb)], sem_o.at[bp])

        def finalize(bp):
            o_copy(bp).start()

        x_copy(0, 0).start()
        x_copy(1, 0).start()
        for piece in range(nbp):
            for c in w_piece_copies(0, 0, piece):
                c.start()
        for c in kv_copies(0, 0):
            c.start()
        q_c[...] = jnp.zeros(q_c.shape, q_c.dtype)
        s_c[...] = jnp.zeros(s_c.shape, s_c.dtype)
        o_c[...] = jnp.zeros(o_c.shape, o_c.dtype)
        acc_s[1, B] = jnp.zeros((Sq, D), f32)
        acc_s[0, B] = jnp.zeros((Sq, D), f32)

        tasks = [(j, w, h) for j in range(bb) for w in range(2) for h in range(hb)]
        T = len(tasks)

        def make_stages(ctx, q, s, p, l, o, not_first, with_acc_store=True):
            def S1(t):
                j, w, h, slot, wslot, b = ctx(t)
                q[t] = jnp.dot(x_s[w, b], wq_s[wslot, w, :, h * Dh:(h + 1) * Dh],
                               preferred_element_type=f32).astype(bf16)

            def S2(t):
                j, w, h, slot, wslot, b = ctx(t)
                s[t] = lax.dot_general(q.pop(t), k_s[slot, w, j, h], (((1,), (1,)), ((), ())),
                                       preferred_element_type=f32)

            def S3(t):
                st = s.pop(t)
                m = jnp.max(st, axis=-1, keepdims=True)
                pt = jnp.exp2((st - m) * (scale * LOG2E))
                l[t] = jnp.sum(pt, axis=-1, keepdims=True)
                p[t] = pt.astype(bf16)

            def S4(t):
                j, w, h, slot, wslot, b = ctx(t)
                ot = jnp.dot(p.pop(t), v_s[slot, w, j, h], preferred_element_type=f32)
                lt = l.pop(t)
                r = pl.reciprocal(lt, approx=True)
                r = r * (2.0 - lt * r)
                o[t] = (ot * r).astype(bf16)

            def S5(t):
                j, w, h, slot, wslot, b = ctx(t)
                c = jnp.dot(o.pop(t), wo_s[wslot, w, h * Dh:(h + 1) * Dh, :],
                            preferred_element_type=f32)
                if h == 0:
                    assert t >= 0
                    new = jnp.where(not_first, acc_s[w, b], 0.0) + c
                else:
                    new = acc_s[w, b] + c
                if h == hb - 1:
                    o_s[b, :, w * D:(w + 1) * D] = new.astype(o_s.dtype)
                    if with_acc_store:
                        acc_s[w, b] = new
                else:
                    acc_s[w, b] = new
            return S1, S2, S3, S4, S5

        def step_body(step, carry):
            hblk = step >> LB
            bp = step & (nbp - 1)
            slot = step & (NB - 1)
            wslot = hblk & (NW - 1)
            pstep = jnp.maximum(step - 1, 0)
            phblk = pstep >> LB
            pslot = pstep & (NB - 1)
            pwslot = phblk & (NW - 1)
            pbp = pstep & (nbp - 1)

            @pl.when(bp == 0)
            def _():
                w_wait(wslot)

            @pl.when(hblk == 0)
            def _():
                x_copy(0, bp).wait()
                x_copy(1, bp).wait()

            for c in kv_copies(step, slot):
                c.wait()

            @pl.when(step + 1 < nsteps)
            def _():
                for c in kv_copies(step + 1, (step + 1) & (NB - 1)):
                    c.start()

            @pl.when(jnp.logical_and(hblk == 0, bp + 1 < nbp))
            def _():
                x_copy(0, bp + 1).start()
                x_copy(1, bp + 1).start()

            @pl.when(hblk + 1 < nh)
            def _():
                for c in w_piece_copies(hblk + 1, (hblk + 1) & (NW - 1), bp):
                    c.start()

            def ctx(t):
                if t < 0:
                    j, w, h = tasks[T + t]
                    pb = jnp.where(step == 0, B, pbp * bb + j)
                    return (j, w, h, pslot, pwslot, pb)
                j, w, h = tasks[t]
                return (j, w, h, slot, wslot, bp * bb + j)

            q = {-1: q_c[...]}; s = {-2: s_c[...]}; p = {}; l = {}; o = {-3: o_c[...]}
            S1, S2, S3, S4, S5 = make_stages(ctx, q, s, p, l, o, hblk > 0)
            for i in range(T):
                S1(i); S2(i - 1); S3(i - 2); S4(i - 2); S5(i - 3)
            q_c[...] = q.pop(T - 1)
            s_c[...] = s.pop(T - 2)
            o_c[...] = o.pop(T - 3)

            @pl.when(jnp.logical_and(step > 0, phblk == nh - 1))
            def _():
                finalize(pbp)

            return carry

        lax.fori_loop(0, nsteps, step_body, 0)

        last = nsteps - 1

        def ctx_l(t):
            j, w, h = tasks[T + t]
            return (j, w, h, last % NB, (nh - 1) % NW, (nbp - 1) * bb + j)

        q = {-1: q_c[...]}; s = {-2: s_c[...]}; p = {}; l = {}; o = {-3: o_c[...]}
        S1, S2, S3, S4, S5 = make_stages(ctx_l, q, s, p, l, o, True, False)
        S2(-1); S3(-2); S4(-2); S5(-3)
        S3(-1); S4(-1); S5(-2)
        S5(-1)
        finalize(nbp - 1)

        for bp in range(nbp):
            o_copy(bp).wait()

    any_spec = pl.BlockSpec(memory_space=pl.ANY)
    return pl.pallas_call(
        kernel,
        in_specs=[any_spec] * 10,
        out_specs=any_spec,
        out_shape=jax.ShapeDtypeStruct((B, Sq, 2 * D), A_x.dtype),
        scratch_shapes=[
            pltpu.VMEM((2, B, Sq, D), bf16),
            pltpu.VMEM((NW, 2, D, hb * Dh), bf16),
            pltpu.VMEM((NW, 2, hb * Dh, D), bf16),
            pltpu.VMEM((NB, 2, bb, hb, Sk, Dh), bf16),
            pltpu.VMEM((NB, 2, bb, hb, Sk, Dh), bf16),
            pltpu.VMEM((2, B + 1, Sq, D), f32),
            pltpu.VMEM((B + 1, Sq, 2 * D), bf16),
            pltpu.VMEM((Sq, Dh), bf16),
            pltpu.VMEM((Sq, Sk), f32),
            pltpu.VMEM((Sq, Dh), bf16),
            pltpu.SemaphoreType.DMA((2, nbp)),
            pltpu.SemaphoreType.DMA((NW, 4)),
            pltpu.SemaphoreType.DMA((NB, 4)),
            pltpu.SemaphoreType.DMA((nbp,)),
        ],
        compiler_params=pltpu.CompilerParams(
            vmem_limit_bytes=100 * 1024 * 1024, disable_bounds_checks=True,
        ),
    )(A_x, A_k_cache, A_v_cache, A_wq, A_wo, B_x, B_k_cache, B_v_cache, B_wq, B_wo)
```
